```python
import os as _os
_os.environ.setdefault("JAX_PLATFORMS", "cpu")
import jax
import jax.numpy as jnp

def _softmax(x, axis=-1):
    return jax.nn.softmax(x, axis=axis)
def _gelu(x):
    return jax.nn.gelu(x, approximate=True)
def _silu(x):
    return jax.nn.silu(x)
def _sigmoid(x):
    return jax.nn.sigmoid(x)
def _layernorm(x, axis=-1, eps=1e-5):
    m = jnp.mean(x, axis=axis, keepdims=True)
    v = jnp.var(x, axis=axis, keepdims=True)
    return (x - m) / jnp.sqrt(v + eps)
def _scatter_add(tgt, idx, src, axis=0):
    return tgt.at[idx].add(src)
def _segment_sum(src, seg, n):
    return jax.ops.segment_sum(src, seg, n)
class _Rng:
    def __init__(self, key):
        self._k = key
    def _next(self):
        self._k, sub = jax.random.split(self._k)
        return sub
    def normal(self, shape):
        return jax.random.normal(self._next(), shape, dtype=jnp.bfloat16)
    def randint(self, lo, hi, shape):
        return jax.random.randint(self._next(), shape, lo, hi, dtype=jnp.int32)
    def uniform(self, shape, lo=0.0, hi=1.0):
        return jax.random.uniform(self._next(), shape, jnp.bfloat16, lo, hi)
    def permutation(self, n):
        return jax.random.permutation(self._next(), n)


kernel_name = 'concat_heads__sliding_local_dilated__linear_attn_block__prompt'

def setup_inputs():
    _rng = _Rng(jax.random.key(int.from_bytes(__import__("os").urandom(4), "little")))
    _w = (lambda a: (lambda t: t.astype(jnp.bfloat16) if jnp.issubdtype(t.dtype, jnp.floating) else t)(jnp.asarray(a)))
    def _A_setup():
        B, S, D = 1, 2048, 640
        return {
            "x": _w((lambda *s: _rng.normal(s) * 0.2)(B, S, D)),
            "wqkv": _w((lambda *s: _rng.normal(s) * 0.2)(D, 3 * D)),
            "wo": _w((lambda *s: _rng.normal(s) * 0.05)(D, D)),
        }
    _A_in = _A_setup()

    def _B_setup():
        B, S, D = 1, 2048, 640
        return {
            "x": _w((lambda *s: _rng.normal(s) * 0.05)(B, S, D)),
            "wqkv": _w((lambda *s: _rng.normal(s) * 1.6)(D, 3 * D)),
            "wo": _w((lambda *s: _rng.normal(s) * 0.4)(D, D)),
        }
    _B_in = _B_setup()

    return {
        "A_x": _A_in["x"],
        "A_wqkv": _A_in["wqkv"],
        "A_wo": _A_in["wo"],
        "B_x": _B_in["x"],
        "B_wqkv": _B_in["wqkv"],
        "B_wo": _B_in["wo"],
    }

def reference(A_x, A_wqkv, A_wo, B_x, B_wqkv, B_wo):
    def _A_ref(x, wqkv, wo):
        B, S, D = x.shape
        H = 32; Dh = D // H
        W, dil = 8, 2
        qkv = (lambda x, *d: x.transpose(*d))((x @ wqkv).reshape(B, S, 3, H, Dh), 2, 0, 3, 1, 4)
        q, k, v = qkv[0], qkv[1], qkv[2]
        scale = Dh ** -0.5
        pos = jnp.arange(S)
        off = jnp.arange(W) * dil
        idx = pos[:, None] - off[None, :]
        mask = idx >= 0
        idx_c = jnp.where(mask, idx, 0).reshape(-1)
        kg = k[:, :, idx_c, :].reshape(B, H, S, W, Dh)
        vg = v[:, :, idx_c, :].reshape(B, H, S, W, Dh)
        logits = jnp.einsum("bhsd,bhswd->bhsw", q, kg) * scale
        logits = jnp.where(mask[None, None, :, :], logits, -1e9)
        attn = _softmax(logits, axis=-1)
        o = jnp.einsum("bhsw,bhswd->bhsd", attn, vg)
        return (lambda x, *d: x.transpose(*d))(o, 0, 2, 1, 3).reshape(B, S, D) @ wo

    def _B_ref(x, wqkv, wo):
        B, S, D = x.shape
        H = 32; Dh = D // H
        qkv = (lambda x, *d: x.transpose(*d))((x @ wqkv).reshape(B, S, 3, H, Dh), 2, 0, 3, 1, 4)
        q, k, v = qkv[0], qkv[1], qkv[2]
        phi = lambda t: jnp.where(t > 0, t + 1, jnp.exp(t)) + 1e-6
        pq, pk = phi(q), phi(k)
        kv = jnp.einsum("bhsd,bhse->bhde", pk, v)
        z = jnp.einsum("bhsd->bhd", pk)
        num = jnp.einsum("bhqd,bhde->bhqe", pq, kv)
        den = jnp.einsum("bhqd,bhd->bhq", pq, z)[..., None] + 1e-6
        o = num / den
        return (lambda x, *d: x.transpose(*d))(o, 0, 2, 1, 3).reshape(B, S, D) @ wo

    a = _A_ref(A_x, A_wqkv, A_wo)
    b = _B_ref(B_x, B_wqkv, B_wo)
    return jnp.concatenate([a, b], axis=-1)
```

```python
import functools
import math

import jax
import jax.numpy as jnp
import jax.experimental.pallas as pl
import jax.experimental.pallas.tpu as pltpu

S = 2048
D = 640
H = 32
DH = 20
W = 8
DIL = 2
NT = D // 128
TA = 256
TB = 512
HALO = 16
CH = 16
F32 = jnp.float32
BF16 = jnp.bfloat16
NT_DIMS = (((1,), (1,)), ((), ()))
EXP2_SCALE = (DH ** -0.5) * math.log2(math.e)


def _phi(t):
    return jnp.where(t > 0, t + 1.0, jnp.exp(t)) + 1e-6


def _group_sum(p):
    p = p + pltpu.roll(p, 64, 1)
    return p + pltpu.roll(p, 32, 1)


def _kernel(ax_hbm, awqkv_hbm, awo_hbm, bx_hbm, bwqkv_hbm, bwo_hbm, out_hbm,
            ax_v, bx_v, awqkv_v, awo_v, bwqkv_v, bwo_v,
            a_wt, a_wo, b_wqt, b_wkt, b_m,
            tmp, q_s, k_s, v_s, o_s, g_s, z_s, zrow, out_v,
            in_sems, out_sems):
    def cp(src, dst, i):
        return pltpu.make_async_copy(src, dst, in_sems.at[i])

    c_bwk = cp(bwqkv_hbm.at[:, D:2 * D], bwqkv_v.at[:, D:2 * D], 0)
    c_bx = [cp(bx_hbm.at[pl.ds(i * TB, TB)], bx_v.at[pl.ds(i * TB, TB)], 1 + i) for i in range(4)]
    c_aw = [cp(awqkv_hbm.at[:, j * D:(j + 1) * D], awqkv_v.at[:, j * D:(j + 1) * D], 5 + j) for j in range(3)]
    c_ax = [cp(ax_hbm.at[pl.ds(i * TB, TB)], ax_v.at[pl.ds(i * TB, TB)], 8 + i) for i in range(4)]
    c_awo = cp(awo_hbm, awo_v, 12)
    c_bwv = cp(bwqkv_hbm.at[:, 2 * D:3 * D], bwqkv_v.at[:, 2 * D:3 * D], 13)
    c_bwq = cp(bwqkv_hbm.at[:, 0:D], bwqkv_v.at[:, 0:D], 14)
    c_bwo = cp(bwo_hbm, bwo_v, 15)
    order = [c_bwk, c_bx[0], c_aw[0], c_aw[1], c_aw[2], c_ax[0], c_awo, c_bx[1], c_bx[2],
             c_ax[1], c_bx[3], c_bwv, c_bwo, c_bwq, c_ax[2], c_ax[3]]
    for c in order:
        c.start()

    def out_copy_a(r0, i):
        return pltpu.make_async_copy(out_v.at[pl.ds(r0, TA), 0:D], out_hbm.at[pl.ds(r0, TA), 0:D],
                                     out_sems.at[i])

    def out_copy_b(r0, i):
        return pltpu.make_async_copy(out_v.at[pl.ds(r0, TB), D:2 * D], out_hbm.at[pl.ds(r0, TB), D:2 * D],
                                     out_sems.at[8 + i])

    def permute_rows_from_tmp(dst, row0):
        for d in range(DH):
            for t in range(NT):
                dst[row0 + d * H:row0 + (d + 1) * H, t * 128:(t + 1) * 128] = (
                    tmp[t, pl.ds(d, H, stride=DH), :].astype(dst.dtype))

    def to_tmp(val):
        for t in range(NT):
            tmp[t] = val[:, t * 128:(t + 1) * 128]

    def prep_transposed(src, dst, row0):
        to_tmp(src.astype(F32).T)
        permute_rows_from_tmp(dst, row0)

    def b_pass1(r0, first):
        x = bx_v[pl.ds(r0, TB), :]
        kt = jax.lax.dot_general(b_wkt[...], x, NT_DIMS, preferred_element_type=F32)
        pk = _phi(kt)
        zp = pk[:, 0:128]
        for j in range(1, TB // 128):
            zp = zp + pk[:, j * 128:(j + 1) * 128]
        g = jnp.dot(pk.astype(BF16), x, preferred_element_type=F32)
        if first:
            z_s[...] = zp
            g_s[...] = g
        else:
            z_s[...] += zp
            g_s[...] += g

    def a_qkv(r0):
        x = ax_v[pl.ds(r0, TA), :]
        qkv = jax.lax.dot_general(x, a_wt[...], NT_DIMS, preferred_element_type=F32)
        for t in range(NT):
            q_s[t] = qkv[:, t * 128:(t + 1) * 128]
            k_s[t, HALO:HALO + TA, :] = qkv[:, D + t * 128:D + (t + 1) * 128]
            v_s[t, HALO:HALO + TA, :] = qkv[:, 2 * D + t * 128:2 * D + (t + 1) * 128]

    def a_attn(r0):
        for c in range(TA // CH):
            c0 = c * CH
            q = [q_s[t, c0:c0 + CH, :] for t in range(NT)]
            logits = []
            for w in range(W):
                off = HALO + c0 - DIL * w
                p = q[0] * k_s[0, off:off + CH, :]
                for t in range(1, NT):
                    p = p + q[t] * k_s[t, off:off + CH, :]
                l = _group_sum(p)
                if c0 < HALO and w > 0:
                    pos = r0 + c0 + jax.lax.broadcasted_iota(jnp.int32, (CH, 128), 0)
                    l = jnp.where(pos >= DIL * w, l, -1e30)
                logits.append(l)
            m = logits[0]
            for w in range(1, W):
                m = jnp.maximum(m, logits[w])
            e = [jnp.exp2((l - m) * EXP2_SCALE) for l in logits]
            den = e[0]
            for w in range(1, W):
                den = den + e[w]
            r = 1.0 / den
            for t in range(NT):
                acc = e[0] * v_s[t, HALO + c0:HALO + c0 + CH, :]
                for w in range(1, W):
                    off = HALO + c0 - DIL * w
                    acc = acc + e[w] * v_s[t, off:off + CH, :]
                o_s[c0:c0 + CH, t * 128:(t + 1) * 128] = (acc * r).astype(BF16)
        for t in range(NT):
            k_s[t, 0:HALO, :] = k_s[t, TA:TA + HALO, :]
            v_s[t, 0:HALO, :] = v_s[t, TA:TA + HALO, :]

    def a_out(r0):
        out_v[pl.ds(r0, TA), 0:D] = jnp.dot(o_s[...], a_wo[...], preferred_element_type=F32).astype(BF16)

    def b_switch():
        bounds = []
        for j in range(NT):
            h0 = (128 * j) // DH
            h1 = (128 * j + 127) // DH
            lo = (h0 * DH) // 16 * 16
            hi = -(-((h1 + 1) * DH) // 16) * 16
            bounds.append((lo, hi))
        for t in range(NT):
            tmp[t] = jnp.zeros((D, 128), F32)
        for j, (lo, hi) in enumerate(bounds):
            gj = g_s[lo:hi, :].astype(BF16)
            kv = jnp.dot(gj, bwqkv_v[:, 2 * D + j * 128:2 * D + (j + 1) * 128], preferred_element_type=F32)
            rh = (lo + jax.lax.broadcasted_iota(jnp.int32, kv.shape, 0)) // DH
            ch = (j * 128 + jax.lax.broadcasted_iota(jnp.int32, kv.shape, 1)) // DH
            kv = jnp.where(rh == ch, kv, 0.0).astype(BF16)
            mj = jnp.dot(kv, bwo_v[j * 128:(j + 1) * 128, :], preferred_element_type=F32)
            for t in range(NT):
                tmp[t, lo:hi, :] += mj[:, t * 128:(t + 1) * 128]
        permute_rows_from_tmp(b_m, 0)
        zp = jnp.concatenate([z_s[pl.ds(d, H, stride=DH), :] for d in range(DH)], axis=0)
        z = jnp.sum(zp.T, axis=0, keepdims=True)
        zrow[...] = jnp.broadcast_to(z, zrow.shape)

    def b_pass2(r0):
        x = bx_v[pl.ds(r0, TB), :]
        q = jax.lax.dot_general(x, b_wqt[...], NT_DIMS, preferred_element_type=F32)
        pq = _phi(q)
        z = zrow[0:1, :]
        p = pq[:, 0:128] * z[:, 0:128]
        for t in range(1, NT):
            p = p + pq[:, t * 128:(t + 1) * 128] * z[:, t * 128:(t + 1) * 128]
        r = 1.0 / (_group_sum(p) + 1e-6)
        pqn = jnp.concatenate([pq[:, t * 128:(t + 1) * 128] * r for t in range(NT)], axis=1).astype(BF16)
        out_v[pl.ds(r0, TB), D:2 * D] = jnp.dot(pqn, b_m[...], preferred_element_type=F32).astype(BF16)

    for t in range(NT):
        k_s[t, 0:HALO, :] = jnp.zeros((HALO, 128), F32)
        v_s[t, 0:HALO, :] = jnp.zeros((HALO, 128), F32)

    c_bwk.wait()
    b_wkt[...] = bwqkv_v[:, D:2 * D].T
    c_bx[0].wait()
    b_pass1(0, True)
    for j in range(3):
        c_aw[j].wait()
        prep_transposed(awqkv_v[:, j * D:(j + 1) * D], a_wt, j * D)
    c_awo.wait()
    to_tmp(awo_v[...].astype(F32))
    permute_rows_from_tmp(a_wo, 0)
    for c in (c_ax[0], c_bx[1], c_bx[2], c_ax[1], c_bx[3]):
        c.wait()

    def loop1(i, carry):
        ra = pl.multiple_of(i * TA, TA)
        rb = pl.multiple_of((i + 1) * TB, TB)
        a_qkv(ra)
        b_pass1(rb, False)
        a_attn(ra)
        a_out(ra)
        out_copy_a(ra, i).start()
        return carry

    jax.lax.fori_loop(0, 3, loop1, 0)

    for c in (c_bwv, c_bwo, c_bwq, c_ax[2], c_ax[3]):
        c.wait()
    a_qkv(3 * TA)
    b_switch()
    prep_transposed(bwqkv_v[:, 0:D], b_wqt, 0)
    a_attn(3 * TA)
    a_out(3 * TA)
    out_copy_a(3 * TA, 3).start()

    def loop2(i, carry):
        ra = pl.multiple_of((i + 4) * TA, TA)
        rb = pl.multiple_of(i * TB, TB)
        a_qkv(ra)
        b_pass2(rb)
        a_attn(ra)
        a_out(ra)
        out_copy_a(ra, i + 4).start()
        out_copy_b(rb, i).start()
        return carry

    jax.lax.fori_loop(0, 4, loop2, 0)

    for i in range(8):
        out_copy_a(i * TA, i).wait()
    for i in range(4):
        out_copy_b(i * TB, i).wait()


@jax.jit
def pallas_concat_heads__sliding_local_dilated__linear_attn_block__prompt_kernel(A_x, A_wqkv, A_wo, B_x, B_wqkv, B_wo):
    any_spec = pl.BlockSpec(memory_space=pl.ANY)
    out = pl.pallas_call(
        _kernel,
        out_shape=jax.ShapeDtypeStruct((S, 2 * D), BF16),
        in_specs=[any_spec] * 6,
        out_specs=any_spec,
        scratch_shapes=[
            pltpu.VMEM((S, D), BF16), pltpu.VMEM((S, D), BF16),
            pltpu.VMEM((D, 3 * D), BF16), pltpu.VMEM((D, D), BF16),
            pltpu.VMEM((D, 3 * D), BF16), pltpu.VMEM((D, D), BF16),
            pltpu.VMEM((3 * D, D), BF16), pltpu.VMEM((D, D), BF16),
            pltpu.VMEM((D, D), BF16), pltpu.VMEM((D, D), BF16), pltpu.VMEM((D, D), BF16),
            pltpu.VMEM((NT, D, 128), F32),
            pltpu.VMEM((NT, TA, 128), F32),
            pltpu.VMEM((NT, HALO + TA, 128), F32), pltpu.VMEM((NT, HALO + TA, 128), F32),
            pltpu.VMEM((TA, D), BF16),
            pltpu.VMEM((D, D), F32), pltpu.VMEM((D, 128), F32), pltpu.VMEM((8, D), F32),
            pltpu.VMEM((S, 2 * D), BF16),
            pltpu.SemaphoreType.DMA((16,)), pltpu.SemaphoreType.DMA((12,)),
        ],
        compiler_params=pltpu.CompilerParams(vmem_limit_bytes=100 * 1024 * 1024),
    )(A_x.reshape(S, D), A_wqkv, A_wo, B_x.reshape(S, D), B_wqkv, B_wo)
    return out.reshape(1, S, 2 * D)
```

```python
import math

import jax
import jax.numpy as jnp
import jax.experimental.pallas as pl
import jax.experimental.pallas.tpu as pltpu

S = 2048
D = 640
H = 32
DH = 20
W = 8
DIL = 2
NT = D // 128
TA = 256
TB1 = 512
HALO = 16
TA2 = 224
NSUB = 4
BUF = NSUB * TA2
WA = 384
XA = 256
CH = 8
OSPLIT = 64
F32 = jnp.float32
BF16 = jnp.bfloat16
U32 = jnp.uint32
NT_DIMS = (((1,), (1,)), ((), ()))
LOG2E = math.log2(math.e)
EXP2_SCALE = (DH ** -0.5) * LOG2E


def _gate(tok, value):
    return jnp.where(tok > jnp.inf, value + 1, value)


def _phi(t):
    return jnp.where(t > 0, t + 1.0, jnp.exp(t)) + 1e-6


def _group_sum(p):
    return (p + pltpu.roll(p, 64, 1)) + (pltpu.roll(p, 32, 1) + pltpu.roll(p, 96, 1))


def _ld(ref, r0, r1):
    return jnp.concatenate([ref[t, r0:r1, :] for t in range(NT)], axis=1)


def _rows(r0, n):
    return pl.ds(r0 if isinstance(r0, int) else pl.multiple_of(r0, 16), n)


def _pack2(a, b):
    lo = jax.lax.bitcast_convert_type(a.astype(F32), U32) >> 16
    return lo | jax.lax.bitcast_convert_type(b.astype(F32), U32)


def _unpack2(x):
    a = jax.lax.bitcast_convert_type(x << 16, F32)
    b = jax.lax.bitcast_convert_type(x & jnp.uint32(0xFFFF0000), F32)
    return a.astype(BF16), b.astype(BF16)


def _kernel(ax_hbm, awqkv_hbm, awo_hbm, bx_hbm, bwqkv_hbm, bwo_hbm, out_hbm,
            ax_v, bx_v, raw,
            wt, a_wo, b_wkt, b_m,
            tmp_m, tmp_t, tmp_w, qkv_s, o_s, g_s, z_s, zrow, out_v,
            in_sems, out_sems):
    q_s = qkv_s.at[0:NT]
    k_s = qkv_s.at[NT:2 * NT]
    v_s = qkv_s.at[2 * NT:3 * NT]

    def cp(src, dst, i):
        return pltpu.make_async_copy(src, dst, in_sems.at[i])

    def c_bx(i):
        return cp(bx_hbm.at[_rows(i * TB1, TB1)], bx_v.at[_rows(i * TB1, TB1)], i)

    def c_wo(i):
        return cp(awo_hbm.at[_rows(i * (D // 2), D // 2)], raw.at[5, _rows(i * (D // 2), D // 2)], 16 + i)

    raw_src = {1: awqkv_hbm.at[:, 0:D], 2: awqkv_hbm.at[:, D:2 * D], 3: awqkv_hbm.at[:, 2 * D:3 * D],
               4: bwqkv_hbm.at[:, 0:D], 6: bwqkv_hbm.at[:, 2 * D:3 * D], 7: bwo_hbm}
    c_raw = {k: cp(src, raw.at[k], 4 + k) for k, src in raw_src.items()}
    c_wka = cp(bwqkv_hbm.at[:, D:D + WA], raw.at[0, :, 0:WA], 0)
    c_wkb = cp(bwqkv_hbm.at[:, D + WA:2 * D], raw.at[0, :, WA:D], 4)
    c_xa = cp(bx_hbm.at[0:XA], bx_v.at[0:XA], 14)
    c_xb = cp(bx_hbm.at[XA:TB1], bx_v.at[XA:TB1], 15)
    c_ax0 = cp(ax_hbm.at[0:TA], ax_v.at[0:TA], 12)
    c_ax1 = cp(ax_hbm.at[TA:S], ax_v.at[TA:S], 13)
    for c in [c_wka, c_xa, c_wkb, c_xb, c_bx(1), c_raw[1], c_raw[2], c_wo(0), c_bx(2), c_raw[3], c_raw[4],
              c_wo(1), c_bx(3), c_raw[6], c_raw[7], c_ax0, c_ax1]:
        c.start()
    a_wt0 = 0
    b_wq0 = 3 * D

    def out_copy(r0, rows, col0, sem, ov=out_v, oh=out_hbm):
        return pltpu.make_async_copy(ov.at[r0:r0 + rows, col0:col0 + D],
                                     oh.at[r0:r0 + rows, col0:col0 + D], out_sems.at[sem])

    def pace(v, n):
        z = _gate(v.astype(F32)[0:8], jnp.uint32(0))
        return jnp.concatenate([z] * n, axis=0)

    def prep_pair(ka, kb, row_a, row_b):
        for t in range(NT):
            rows = slice(t * 128, (t + 1) * 128)
            tmp_t[...] = _pack2(raw[ka, rows, :], raw[kb, rows, :]).T
            for d in range(DH):
                x = tmp_t[pl.ds(d, H, stride=DH), :]
                if (t or d) and d % 4 == 0:
                    x = x | pace(wt[0, _rows(row_a, 16), :], H // 8)
                a, b = _unpack2(x)
                wt[t, _rows(row_a + d * H, H), :] = a
                wt[t, _rows(row_b + d * H, H), :] = b

    def prep_wo(i):
        hd = D // 2
        w = raw[5, _rows(i * hd, hd), :]
        for p in range(3):
            ta, tb = 2 * p, min(2 * p + 1, NT - 1)
            tmp_w[...] = _pack2(w[:, ta * 128:(ta + 1) * 128], w[:, tb * 128:(tb + 1) * 128])
            for d in range(DH):
                x = tmp_w[pl.ds(d, H // 2, stride=DH), :]
                if (p or d) and d % 5 == 0:
                    x = x | pace(a_wo[0, _rows(i * (H // 2), 16), :], H // 16)
                a, b = _unpack2(x)
                rows = _rows(d * H + i * (H // 2), H // 2)
                a_wo[ta, rows, :] = a
                if tb != ta:
                    a_wo[tb, rows, :] = b

    def wk_transpose(f0, f1):
        wkt = raw[0, :, f0:f1].T
        for t in range(NT):
            b_wkt[t, f0:f1, :] = wkt[:, t * 128:(t + 1) * 128]

    def b1_k(r0, rows, f0=0, f1=D, first=False):
        x = bx_v[_rows(r0, rows), :]
        kt = jax.lax.dot_general(_ld(b_wkt, f0, f1), x, NT_DIMS, preferred_element_type=F32)
        pk = _phi(kt)
        zp = pk[:, 0:128]
        for j in range(1, rows // 128):
            zp = zp + pk[:, j * 128:(j + 1) * 128]
        if first:
            z_s[f0:f1, :] = zp
        else:
            z_s[f0:f1, :] += zp
        return pk.astype(BF16)

    def b1_g(r0, rows, pk, f0=0, f1=D, first=False):
        x = bx_v[_rows(r0, rows), :]
        g = jnp.dot(pk, x, preferred_element_type=F32)
        if first:
            g_s[f0:f1, :] = g
        else:
            g_s[f0:f1, :] += g

    def a_proj(xr, r0, b0, rows):
        y = jax.lax.dot_general(xr[r0:r0 + rows, :], _ld(wt, a_wt0, a_wt0 + 3 * D), NT_DIMS,
                                preferred_element_type=F32)
        for t in range(3 * NT):
            qkv_s[t, HALO + b0:HALO + b0 + rows, :] = y[:, t * 128:(t + 1) * 128]

    def a_attn(b0, rows, first=False):
        tok = None
        for c in range(rows // CH):
            c0 = HALO + b0 + c * CH
            sc = EXP2_SCALE if tok is None else _gate(tok, jnp.float32(EXP2_SCALE))
            q = [q_s[t, c0:c0 + CH, :] * sc for t in range(NT)]
            logits = []
            for w in range(W):
                off = c0 - DIL * w
                p = q[0] * k_s[0, off:off + CH, :]
                for t in range(1, NT):
                    p = p + q[t] * k_s[t, off:off + CH, :]
                l = _group_sum(p)
                if first and c * CH < HALO and w > 0:
                    pos = c * CH + jax.lax.broadcasted_iota(jnp.int32, (CH, 128), 0)
                    l = jnp.where(pos >= DIL * w, l, -1e30)
                logits.append(l)
            tok = logits[0]
            m = logits[0]
            for w in range(1, W):
                m = jnp.maximum(m, logits[w])
            e = [jnp.exp2(l - m) for l in logits]
            den = e[0]
            for w in range(1, W):
                den = den + e[w]
            r = 1.0 / den
            for t in range(NT):
                acc = e[0] * v_s[t, c0:c0 + CH, :]
                for w in range(1, W):
                    off = c0 - DIL * w
                    acc = acc + e[w] * v_s[t, off:off + CH, :]
                o_s[t, c0 - HALO:c0 - HALO + CH, :] = (acc * r).astype(BF16)

    def a_out(r0, b0, rows, sem, ov=out_v, oh=out_hbm):
        ov[r0:r0 + rows, 0:D] = jnp.dot(_ld(o_s, b0, b0 + rows), _ld(a_wo, 0, D),
                                        preferred_element_type=F32).astype(BF16)
        out_copy(r0, rows, 0, sem, ov, oh).start()

    def carry_halo():
        for t in range(NT):
            k_s[t, 0:HALO, :] = k_s[t, BUF:BUF + HALO, :]
            v_s[t, 0:HALO, :] = v_s[t, BUF:BUF + HALO, :]

    bounds = []
    for j in range(NT):
        h0 = (128 * j) // DH
        h1 = (128 * j + 127) // DH
        bounds.append(((h0 * DH) // 16 * 16, -(-((h1 + 1) * DH) // 16) * 16))

    def b_switch():
        zp = jnp.concatenate([z_s[pl.ds(d, H, stride=DH), :] for d in range(DH)], axis=0)
        zrow[...] = jnp.broadcast_to(jnp.sum(zp.T, axis=0, keepdims=True), zrow.shape)
        kvs = []
        for j, (lo, hi) in enumerate(bounds):
            kv = jnp.dot(g_s[lo:hi, :].astype(BF16), raw[6, :, j * 128:(j + 1) * 128],
                         preferred_element_type=F32)
            row = lo + jax.lax.broadcasted_iota(jnp.int32, kv.shape, 0)
            head0 = (j * 128 + jax.lax.broadcasted_iota(jnp.int32, (1, 128), 1)) // DH * DH
            same_head = jnp.logical_and(row >= head0, row < head0 + DH)
            kvs.append(jnp.where(same_head, kv, 0.0).astype(BF16))
        done = 0
        for j, (lo, hi) in enumerate(bounds):
            mj = jnp.dot(kvs[j], raw[7, j * 128:(j + 1) * 128, :], preferred_element_type=F32)
            for t in range(NT):
                mt = mj[:, t * 128:(t + 1) * 128]
                if done > lo:
                    tmp_m[t, lo:done, :] += mt[0:done - lo]
                tmp_m[t, max(done, lo):hi, :] = mt[max(done, lo) - lo:]
            done = hi
        for t in range(NT):
            for d in range(DH):
                b_m[t, d * H:(d + 1) * H, :] = tmp_m[t, pl.ds(d, H, stride=DH), :].astype(BF16)

    def b2_q(xr, r0):
        q = jax.lax.dot_general(xr[r0:r0 + TA, :], _ld(wt, b_wq0, b_wq0 + D), NT_DIMS,
                                preferred_element_type=F32)
        z = zrow[...]
        dens, out = [], []
        for c in range(TA // CH):
            l2e = LOG2E if c < 2 else _gate(dens[c - 2], jnp.float32(LOG2E))
            pq = []
            for t in range(NT):
                qt = q[c * CH:(c + 1) * CH, t * 128:(t + 1) * 128]
                pq.append(jnp.where(qt > 0, qt + 1.0, jnp.exp2(qt * l2e)) + 1e-6)
            p = pq[0] * z[:, 0:128]
            for t in range(1, NT):
                p = p + pq[t] * z[:, t * 128:(t + 1) * 128]
            den = _group_sum(p) + 1e-6
            dens.append(den)
            r = 1.0 / den
            out.append(jnp.concatenate([pq[t] * r for t in range(NT)], axis=1))
        return jnp.concatenate(out, axis=0).astype(BF16)

    def b2_out(r0, pqn, sem, ov, oh):
        ov[r0:r0 + TA, D:2 * D] = jnp.dot(pqn, _ld(b_m, 0, D), preferred_element_type=F32).astype(BF16)
        out_copy(r0, TA, D, sem, ov, oh).start()

    b00 = BUF - TA
    hw = WA // 2
    n0 = TA2 - OSPLIT

    def main(_, carry0):
        c_wka.wait()
        wk_transpose(0, WA)
        c_xa.wait()
        pk1 = b1_k(0, XA, 0, hw, True)
        pk2 = b1_k(0, XA, hw, WA, True)
        b1_g(0, XA, pk1, 0, hw, True)
        b1_g(0, XA, pk2, hw, WA, True)
        c_wkb.wait()
        c_xb.wait()
        pk1 = b1_k(XA, TB1 - XA, 0, hw)
        pk2 = b1_k(XA, TB1 - XA, hw, WA)
        wk_transpose(WA, D)
        pk3 = b1_k(0, TB1, WA, D, True)
        b1_g(XA, TB1 - XA, pk1, 0, hw)
        b1_g(XA, TB1 - XA, pk2, hw, WA)
        b1_g(0, TB1, pk3, WA, D, True)

        def b1_loop(i, carry):
            c_bx(i + 1).wait()
            for j in range(2):
                k = 2 * i + 1 + j
                cp(raw.at[k], raw.at[k], 4 + k).wait()
            c_wo(i).wait()
            r0 = (i + 1) * TB1
            pk = b1_k(r0, TB1)
            prep_wo(i)
            prep_pair(2 * i + 1, 2 * i + 2, 2 * i * D, (2 * i + 1) * D)
            b1_g(r0, TB1, pk)
            return carry

        jax.lax.fori_loop(0, 2, b1_loop, 0)

        for c in (c_bx(3), c_raw[6], c_raw[7], c_ax0):
            c.wait()
        pk = b1_k(3 * TB1, TB1)
        for t in range(NT):
            k_s[t, b00:b00 + HALO, :] = jnp.zeros((HALO, 128), F32)
            v_s[t, b00:b00 + HALO, :] = jnp.zeros((HALO, 128), F32)
        a_proj(ax_v, 0, b00, TA)
        b1_g(3 * TB1, TB1, pk)
        b_switch()
        a_attn(b00, TA, first=True)
        a_out(0, b00, TA, 0)
        carry_halo()
        c_ax1.wait()

        def steady(it, carry):
            wa = pl.ds(pl.multiple_of(it * BUF, 128), TA + BUF)
            wb = pl.ds(pl.multiple_of(it * NSUB * TA, 128), NSUB * TA)
            axr, ova, oha = ax_v.at[wa], out_v.at[wa], out_hbm.at[wa]
            bxr, ovb, ohb = bx_v.at[wb], out_v.at[wb], out_hbm.at[wb]
            pqn = {}
            b_work = [[("q", 0), ("q", 1)], [("o", 0), ("q", 2)], [("o", 1), ("q", 3)], [("o", 2), ("o", 3)]]
            for j in range(NSUB):
                ra = TA + j * TA2
                a_proj(axr, ra, j * TA2, TA2)
                for kind, idx in b_work[j]:
                    if kind == "q":
                        pqn[idx] = b2_q(bxr, idx * TA)
                    else:
                        b2_out(idx * TA, pqn.pop(idx), 11 + it * NSUB + idx, ovb, ohb)
                a_attn(j * TA2, TA2)
                sem = 1 + it * (NSUB + 1) + j
                if j + 1 < NSUB:
                    a_out(ra, j * TA2, TA2, sem, ova, oha)
                else:
                    a_out(ra, j * TA2, n0, sem, ova, oha)
                    a_out(ra + n0, j * TA2 + n0, OSPLIT, sem + 1, ova, oha)
            carry_halo()
            return carry

        jax.lax.fori_loop(0, 2, steady, 0)
        return carry0

    jax.lax.fori_loop(0, 1 + pl.program_id(0), main, 0)

    out_copy(0, TA, 0, 0).wait()
    for it in range(2):
        for j in range(NSUB):
            r0 = TA + it * BUF + j * TA2
            sem = 1 + it * (NSUB + 1) + j
            if j + 1 < NSUB:
                out_copy(r0, TA2, 0, sem).wait()
            else:
                out_copy(r0, n0, 0, sem).wait()
                out_copy(r0 + n0, OSPLIT, 0, sem + 1).wait()
    for i in range(2 * NSUB):
        out_copy(i * TA, TA, D, 11 + i).wait()


@jax.jit
def pallas_concat_heads__sliding_local_dilated__linear_attn_block__prompt_kernel(A_x, A_wqkv, A_wo, B_x, B_wqkv, B_wo):
    any_spec = pl.BlockSpec(memory_space=pl.ANY)
    out = pl.pallas_call(
        _kernel,
        out_shape=jax.ShapeDtypeStruct((S, 2 * D), BF16),
        grid=(1,),
        in_specs=[any_spec] * 6,
        out_specs=any_spec,
        scratch_shapes=[
            pltpu.VMEM((S, D), BF16), pltpu.VMEM((S, D), BF16),
            pltpu.VMEM((8, D, D), BF16),
            pltpu.VMEM((NT, 4 * D, 128), BF16), pltpu.VMEM((NT, D, 128), BF16),
            pltpu.VMEM((NT, D, 128), BF16), pltpu.VMEM((NT, D, 128), BF16),
            pltpu.VMEM((NT, D, 128), F32), pltpu.VMEM((D, 128), U32), pltpu.VMEM((D // 2, 128), U32),
            pltpu.VMEM((3 * NT, HALO + BUF, 128), F32),
            pltpu.VMEM((NT, BUF, 128), BF16),
            pltpu.VMEM((D, D), F32), pltpu.VMEM((D, 128), F32), pltpu.VMEM((8, D), F32),
            pltpu.VMEM((S, 2 * D), BF16),
            pltpu.SemaphoreType.DMA((18,)), pltpu.SemaphoreType.DMA((19,)),
        ],
        compiler_params=pltpu.CompilerParams(vmem_limit_bytes=100 * 1024 * 1024,
                                             disable_bounds_checks=True,
                                             disable_semaphore_checks=True),
    )(A_x.reshape(S, D), A_wqkv, A_wo, B_x.reshape(S, D), B_wqkv, B_wo)
    return out.reshape(1, S, 2 * D)
```

```python
import math

import jax
import jax.numpy as jnp
import jax.experimental.pallas as pl
import jax.experimental.pallas.tpu as pltpu

S = 2048
D = 640
H = 32
DH = 20
W = 8
DIL = 2
NT = D // 128
TA = 256
TB1 = 512
HALO = 16
TA2 = 224
NSUB = 4
BUF = NSUB * TA2
WA = 256
XA = 384
CH = 8
OSP = (128, 64, 32)
NO = NSUB - 1 + len(OSP)
PAD = 24
F32 = jnp.float32
BF16 = jnp.bfloat16
U32 = jnp.uint32
NT_DIMS = (((1,), (1,)), ((), ()))
LOG2E = math.log2(math.e)
EXP2_SCALE = (DH ** -0.5) * LOG2E


def _gate(tok, value):
    return jnp.where(tok > jnp.inf, value + 1, value)


def _phi(t):
    return jnp.where(t > 0, t + 1.0, jnp.exp(t)) + 1e-6


def _group_sum(p):
    return (p + pltpu.roll(p, 64, 1)) + (pltpu.roll(p, 32, 1) + pltpu.roll(p, 96, 1))


def _ld(ref, r0, r1):
    return jnp.concatenate([ref[t, r0:r1, :] for t in range(NT)], axis=1)


def _rows(r0, n):
    return pl.ds(r0 if isinstance(r0, int) else pl.multiple_of(r0, 16), n)


def _pack2(a, b):
    lo = jax.lax.bitcast_convert_type(a.astype(F32), U32) >> 16
    return lo | jax.lax.bitcast_convert_type(b.astype(F32), U32)


def _unpack2(x):
    a = jax.lax.bitcast_convert_type(x << 16, F32)
    b = jax.lax.bitcast_convert_type(x & jnp.uint32(0xFFFF0000), F32)
    return a.astype(BF16), b.astype(BF16)


def _kernel(ax_hbm, awqkv_hbm, awo_hbm, bx_hbm, bwqkv_hbm, bwo_hbm, out_hbm,
            ax_v, bx_v, raw, rawp,
            wt, a_wo, b_wkt, b_m,
            tmp_m, tmp_t, tmp_w, qkv_s, o_s, g_s, z_s, zrow, out_v,
            in_sems, out_sems):
    q_s = qkv_s.at[0:NT]
    k_s = qkv_s.at[NT:2 * NT]
    v_s = qkv_s.at[2 * NT:3 * NT]

    def cp(src, dst, i):
        return pltpu.make_async_copy(src, dst, in_sems.at[i])

    def c_bx(i):
        return cp(bx_hbm.at[_rows(i * TB1, TB1)], bx_v.at[_rows(i * TB1, TB1)], i)

    def c_wo(i):
        return cp(awo_hbm.at[_rows(i * (D // 2), D // 2)], raw.at[1, _rows(i * (D // 2), D // 2)], 16 + i)

    c_raw = {2: cp(bwqkv_hbm.at[:, 2 * D:3 * D], raw.at[2], 10), 3: cp(bwo_hbm, raw.at[3], 11)}
    c_pair0 = cp(awqkv_hbm.at[:, 0:2 * D], rawp.at[0], 5)
    c_pair1 = [cp(awqkv_hbm.at[:, 2 * D:3 * D], rawp.at[1, :, 0:D], 6),
               cp(bwqkv_hbm.at[:, 0:D], rawp.at[1, :, D:2 * D], 6)]
    c_wka = cp(bwqkv_hbm.at[:, D:D + WA], raw.at[0, :, 0:WA], 0)
    c_wkb = cp(bwqkv_hbm.at[:, D + WA:2 * D], raw.at[0, :, WA:D], 4)
    c_xa = cp(bx_hbm.at[0:XA], bx_v.at[0:XA], 14)
    c_xb = cp(bx_hbm.at[XA:TB1], bx_v.at[XA:TB1], 15)
    c_ax0 = cp(ax_hbm.at[0:TA], ax_v.at[0:TA], 12)
    c_ax1 = cp(ax_hbm.at[TA:S], ax_v.at[TA:S], 13)
    for c in [c_wka, c_xa, c_wkb, c_xb, c_bx(1), c_pair0, c_wo(0), c_bx(2), c_pair1[0], c_pair1[1],
              c_wo(1), c_bx(3), c_raw[2], c_raw[3], c_ax0, c_ax1]:
        c.start()
    a_wt0 = 0
    b_wq0 = 3 * D

    def out_copy(r0, rows, col0, sem, ov=out_v, oh=out_hbm):
        return pltpu.make_async_copy(ov.at[r0:r0 + rows, col0:col0 + D],
                                     oh.at[r0:r0 + rows, col0:col0 + D], out_sems.at[sem])

    def pace(v, n):
        z = _gate(v.astype(F32)[0:8], jnp.uint32(0))
        return jnp.concatenate([z] * n, axis=0)

    def prep_pair(k, row_a, row_b):
        for t in range(NT):
            rows = slice(t * 128, (t + 1) * 128)
            tmp_t[0:D, :] = _pack2(rawp[k, rows, 0:D], rawp[k, rows, D:2 * D]).T
            for d in range(DH):
                x = tmp_t[pl.ds(d, H, stride=DH), :]
                if (t or d) and d % 4 == 0:
                    x = x | pace(wt[0, _rows(row_a, 16), :], H // 8)
                a, b = _unpack2(x)
                wt[t, _rows(row_a + d * H, H), :] = a
                wt[t, _rows(row_b + d * H, H), :] = b

    def prep_wo(i):
        hd = D // 2
        w = raw[1, _rows(i * hd, hd), :]
        for p in range(3):
            ta, tb = 2 * p, min(2 * p + 1, NT - 1)
            tmp_w[0:hd, :] = _pack2(w[:, ta * 128:(ta + 1) * 128], w[:, tb * 128:(tb + 1) * 128])
            for d in range(DH):
                x = tmp_w[pl.ds(d, H // 2, stride=DH), :]
                if (p or d) and d % 5 == 0:
                    x = x | pace(a_wo[0, _rows(i * (H // 2), 16), :], H // 16)
                a, b = _unpack2(x)
                rows = _rows(d * H + i * (H // 2), H // 2)
                a_wo[ta, rows, :] = a
                if tb != ta:
                    a_wo[tb, rows, :] = b

    def wk_transpose(f0, f1):
        wkt = raw[0, :, f0:f1].T
        for t in range(NT):
            b_wkt[t, f0:f1, :] = wkt[:, t * 128:(t + 1) * 128]

    def b1_k(r0, rows, f0=0, f1=D, first=False):
        x = bx_v[_rows(r0, rows), :]
        kt = jax.lax.dot_general(_ld(b_wkt, f0, f1), x, NT_DIMS, preferred_element_type=F32)
        pk = _phi(kt)
        zp = pk[:, 0:128]
        for j in range(1, rows // 128):
            zp = zp + pk[:, j * 128:(j + 1) * 128]
        if first:
            z_s[f0:f1, :] = zp
        else:
            z_s[f0:f1, :] += zp
        return pk.astype(BF16)

    def b1_g(r0, rows, pk, f0=0, f1=D, first=False):
        x = bx_v[_rows(r0, rows), :]
        g = jnp.dot(pk, x, preferred_element_type=F32)
        if first:
            g_s[f0:f1, :] = g
        else:
            g_s[f0:f1, :] += g

    def a_proj(xr, r0, b0, rows):
        y = jax.lax.dot_general(xr[r0:r0 + rows, :], _ld(wt, a_wt0, a_wt0 + 3 * D), NT_DIMS,
                                preferred_element_type=F32)
        for t in range(3 * NT):
            qkv_s[t, HALO + b0:HALO + b0 + rows, :] = y[:, t * 128:(t + 1) * 128]

    def a_attn(b0, rows, pace_on, tok=None, first=False):
        for c in range(rows // CH):
            c0 = HALO + b0 + c * CH
            sc = EXP2_SCALE if tok is None else _gate(tok, jnp.float32(EXP2_SCALE))
            q = [q_s[t, c0:c0 + CH, :] * sc for t in range(NT)]
            logits = []
            for w in range(W):
                off = c0 - DIL * w
                p = q[0] * k_s[0, off:off + CH, :]
                for t in range(1, NT):
                    p = p + q[t] * k_s[t, off:off + CH, :]
                l = _group_sum(p)
                if first and c * CH < HALO and w > 0:
                    pos = c * CH + jax.lax.broadcasted_iota(jnp.int32, (CH, 128), 0)
                    l = jnp.where(pos >= DIL * w, l, -1e9 * LOG2E)
                logits.append(l)
            m = logits[0]
            for w in range(1, W):
                m = jnp.maximum(m, logits[w])
            e = [jnp.exp2(l - m) for l in logits]
            den = e[0]
            for w in range(1, W):
                den = den + e[w]
            r = 1.0 / den
            tok = {"logit": logits[W - 1], "max": m, "den": den}[pace_on]
            for t in range(NT):
                acc = e[0] * v_s[t, c0:c0 + CH, :]
                for w in range(1, W):
                    off = c0 - DIL * w
                    acc = acc + e[w] * v_s[t, off:off + CH, :]
                o_s[t, c0 - HALO:c0 - HALO + CH, :] = (acc * r).astype(BF16)
        return tok

    def a_out(r0, b0, rows, sem, ov=out_v, oh=out_hbm):
        ov[r0:r0 + rows, 0:D] = jnp.dot(_ld(o_s, b0, b0 + rows), _ld(a_wo, 0, D),
                                        preferred_element_type=F32).astype(BF16)
        out_copy(r0, rows, 0, sem, ov, oh).start()

    def carry_halo():
        for t in range(NT):
            k_s[t, 0:HALO, :] = k_s[t, BUF:BUF + HALO, :]
            v_s[t, 0:HALO, :] = v_s[t, BUF:BUF + HALO, :]

    bounds = []
    for j in range(NT):
        h0 = (128 * j) // DH
        h1 = (128 * j + 127) // DH
        bounds.append(((h0 * DH) // 16 * 16, -(-((h1 + 1) * DH) // 16) * 16))

    def b_switch():
        zp = jnp.concatenate([z_s[pl.ds(d, H, stride=DH), :] for d in range(DH)], axis=0)
        zrow[...] = jnp.broadcast_to(jnp.sum(zp.T, axis=0, keepdims=True), zrow.shape)
        kvs = []
        for j, (lo, hi) in enumerate(bounds):
            kv = jnp.dot(g_s[lo:hi, :].astype(BF16), raw[2, :, j * 128:(j + 1) * 128],
                         preferred_element_type=F32)
            row = lo + jax.lax.broadcasted_iota(jnp.int32, kv.shape, 0)
            head0 = (j * 128 + jax.lax.broadcasted_iota(jnp.int32, (1, 128), 1)) // DH * DH
            same_head = jnp.logical_and(row >= head0, row < head0 + DH)
            kvs.append(jnp.where(same_head, kv, 0.0).astype(BF16))
        done = 0
        for j, (lo, hi) in enumerate(bounds):
            mj = jnp.dot(kvs[j], raw[3, j * 128:(j + 1) * 128, :], preferred_element_type=F32)
            for t in range(NT):
                mt = mj[:, t * 128:(t + 1) * 128]
                if done > lo:
                    tmp_m[t, lo:done, :] += mt[0:done - lo]
                tmp_m[t, max(done, lo):hi, :] = mt[max(done, lo) - lo:]
            done = hi
        for t in range(NT):
            for d in range(DH):
                b_m[t, d * H:(d + 1) * H, :] = tmp_m[t, pl.ds(d, H, stride=DH), :].astype(BF16)

    def b2_q(xr, r0):
        q = jax.lax.dot_general(xr[r0:r0 + TA, :], _ld(wt, b_wq0, b_wq0 + D), NT_DIMS,
                                preferred_element_type=F32)
        z = zrow[...]
        dens, out = [], []
        for c in range(TA // CH):
            l2e = LOG2E if c < 2 else _gate(dens[c - 2], jnp.float32(LOG2E))
            pq = []
            for t in range(NT):
                qt = q[c * CH:(c + 1) * CH, t * 128:(t + 1) * 128]
                pq.append(jnp.where(qt > 0, qt + 1.0, jnp.exp2(qt * l2e)) + 1e-6)
            p = pq[0] * z[:, 0:128]
            for t in range(1, NT):
                p = p + pq[t] * z[:, t * 128:(t + 1) * 128]
            den = _group_sum(p) + 1e-6
            dens.append(den)
            r = 1.0 / den
            out.append(jnp.concatenate([pq[t] * r for t in range(NT)], axis=1))
        return jnp.concatenate(out, axis=0).astype(BF16)

    def b2_out(r0, pqn, sem, ov, oh):
        ov[r0:r0 + TA, D:2 * D] = jnp.dot(pqn, _ld(b_m, 0, D), preferred_element_type=F32).astype(BF16)
        out_copy(r0, TA, D, sem, ov, oh).start()

    b00 = BUF - TA
    hw = WA // 2

    def main(_, carry0):
        c_wka.wait()
        wk_transpose(0, WA)
        c_xa.wait()
        pk1 = b1_k(0, XA, 0, hw, True)
        pk2 = b1_k(0, XA, hw, WA, True)
        b1_g(0, XA, pk1, 0, hw, True)
        b1_g(0, XA, pk2, hw, WA, True)
        c_wkb.wait()
        c_xb.wait()
        pk1 = b1_k(XA, TB1 - XA, 0, hw)
        pk2 = b1_k(XA, TB1 - XA, hw, WA)
        wk_transpose(WA, D)
        pk3 = b1_k(0, TB1, WA, D, True)
        b1_g(XA, TB1 - XA, pk1, 0, hw)
        b1_g(XA, TB1 - XA, pk2, hw, WA)
        b1_g(0, TB1, pk3, WA, D, True)

        def b1_loop(i, carry):
            c_bx(i + 1).wait()
            cp(rawp.at[i], rawp.at[i], 5 + i).wait()
            c_wo(i).wait()
            r0 = (i + 1) * TB1
            pk = b1_k(r0, TB1)
            prep_wo(i)
            prep_pair(i, 2 * i * D, (2 * i + 1) * D)
            b1_g(r0, TB1, pk)
            return carry

        jax.lax.fori_loop(0, 2, b1_loop, 0)

        for c in (c_bx(3), c_raw[2], c_raw[3], c_ax0):
            c.wait()
        pk = b1_k(3 * TB1, TB1)
        for t in range(NT):
            k_s[t, b00:b00 + HALO, :] = jnp.zeros((HALO, 128), F32)
            v_s[t, b00:b00 + HALO, :] = jnp.zeros((HALO, 128), F32)
        a_proj(ax_v, 0, b00, TA)
        b1_g(3 * TB1, TB1, pk)
        b_switch()
        a_attn(b00, TA, "max", first=True)
        a_out(0, b00, TA, 0)
        carry_halo()
        c_ax1.wait()

        def steady(it, carry):
            wa = pl.ds(pl.multiple_of(it * BUF, 128), TA + BUF)
            wb = pl.ds(pl.multiple_of(it * NSUB * TA, 128), NSUB * TA)
            axr, ova, oha = ax_v.at[wa], out_v.at[wa], out_hbm.at[wa]
            bxr, ovb, ohb = bx_v.at[wb], out_v.at[wb], out_hbm.at[wb]
            pqn = {}
            b_work = [[("q", 0), ("q", 1)], [("o", 0), ("q", 2)], [("o", 1), ("q", 3)], [("o", 2), ("o", 3)]]

            def emit_out(j):
                ra = TA + j * TA2
                sem = 1 + it * NO + j
                if j + 1 < NSUB:
                    a_out(ra, j * TA2, TA2, sem, ova, oha)
                else:
                    off = 0
                    for k, n in enumerate(OSP):
                        a_out(ra + off, j * TA2 + off, n, sem + k, ova, oha)
                        off += n

            tok = None
            for j in range(NSUB):
                ra = TA + j * TA2
                a_proj(axr, ra, j * TA2, TA2)
                if j > 0:
                    emit_out(j - 1)
                for kind, idx in b_work[j]:
                    if kind == "q":
                        pqn[idx] = b2_q(bxr, idx * TA)
                    else:
                        b2_out(idx * TA, pqn.pop(idx), 1 + 2 * NO + it * NSUB + idx, ovb, ohb)
                tok = a_attn(j * TA2, TA2, "den" if j + 1 < NSUB else "logit", tok)
            emit_out(NSUB - 1)
            carry_halo()
            return carry

        jax.lax.fori_loop(0, 2, steady, 0)
        return carry0

    jax.lax.fori_loop(0, 1 + pl.program_id(0), main, 0)

    out_copy(0, TA, 0, 0).wait()
    for it in range(2):
        for j in range(NSUB):
            r0 = TA + it * BUF + j * TA2
            sem = 1 + it * NO + j
            if j + 1 < NSUB:
                out_copy(r0, TA2, 0, sem).wait()
            else:
                off = 0
                for k, n in enumerate(OSP):
                    out_copy(r0 + off, n, 0, sem + k).wait()
                    off += n
    for i in range(2 * NSUB):
        out_copy(i * TA, TA, D, 1 + 2 * NO + i).wait()


@jax.jit
def pallas_concat_heads__sliding_local_dilated__linear_attn_block__prompt_kernel(A_x, A_wqkv, A_wo, B_x, B_wqkv, B_wo):
    any_spec = pl.BlockSpec(memory_space=pl.ANY)
    out = pl.pallas_call(
        _kernel,
        out_shape=jax.ShapeDtypeStruct((S, 2 * D), BF16),
        grid=(1,),
        in_specs=[any_spec] * 6,
        out_specs=any_spec,
        scratch_shapes=[
            pltpu.VMEM((S, D), BF16), pltpu.VMEM((S, D), BF16),
            pltpu.VMEM((4, D, D), BF16), pltpu.VMEM((2, D, 2 * D), BF16),
            pltpu.VMEM((NT, 4 * D, 128), BF16), pltpu.VMEM((NT, D, 128), BF16),
            pltpu.VMEM((NT, D, 128), BF16), pltpu.VMEM((NT, D, 128), BF16),
            pltpu.VMEM((NT, D + PAD, 128), F32), pltpu.VMEM((D + PAD, 128), U32),
            pltpu.VMEM((D // 2 + PAD, 128), U32),
            pltpu.VMEM((3 * NT, HALO + BUF, 128), F32),
            pltpu.VMEM((NT, BUF, 128), BF16),
            pltpu.VMEM((D, D), F32), pltpu.VMEM((D + PAD, 128), F32), pltpu.VMEM((8, D), F32),
            pltpu.VMEM((S, 2 * D), BF16),
            pltpu.SemaphoreType.DMA((18,)), pltpu.SemaphoreType.DMA((9 + 2 * NO,)),
        ],
        compiler_params=pltpu.CompilerParams(vmem_limit_bytes=100 * 1024 * 1024,
                                             disable_bounds_checks=True,
                                             disable_semaphore_checks=True),
    )(A_x.reshape(S, D), A_wqkv, A_wo, B_x.reshape(S, D), B_wqkv, B_wo)
    return out.reshape(1, S, 2 * D)
```

```python
import math

import jax
import jax.numpy as jnp
import jax.experimental.pallas as pl
import jax.experimental.pallas.tpu as pltpu

S = 2048
D = 640
H = 32
DH = 20
W = 8
DIL = 2
NT = D // 128
TA = 256
TB0 = 640
TB1 = 512
TB3 = S - TB0 - 2 * TB1
HALO = 16
TA2 = 224
NSUB = 4
BUF = NSUB * TA2
WA = 256
XA = 384
CH = 8
OSP = (128, 64, 32)
NO = NSUB - 1 + len(OSP)
PAD = 24
F32 = jnp.float32
BF16 = jnp.bfloat16
U32 = jnp.uint32
NT_DIMS = (((1,), (1,)), ((), ()))
LOG2E = math.log2(math.e)
EXP2_SCALE = (DH ** -0.5) * LOG2E


def _gate(tok, value):
    return jnp.where(tok > jnp.inf, value + 1, value)


def _phi(t):
    return jnp.where(t > 0, t + 1.0, jnp.exp(t)) + 1e-6


def _group_sum(p):
    return (p + pltpu.roll(p, 64, 1)) + (pltpu.roll(p, 32, 1) + pltpu.roll(p, 96, 1))


def _ld(ref, r0, r1):
    return jnp.concatenate([ref[t, r0:r1, :] for t in range(NT)], axis=1)


def _rows(r0, n):
    return pl.ds(r0 if isinstance(r0, int) else pl.multiple_of(r0, 16), n)


def _pack2(a, b):
    lo = jax.lax.bitcast_convert_type(a.astype(F32), U32) >> 16
    return lo | jax.lax.bitcast_convert_type(b.astype(F32), U32)


def _unpack2(x):
    a = jax.lax.bitcast_convert_type(x << 16, F32)
    b = jax.lax.bitcast_convert_type(x & jnp.uint32(0xFFFF0000), F32)
    return a.astype(BF16), b.astype(BF16)


def _kernel(ax_hbm, awqkv_hbm, awo_hbm, bx_hbm, bwqkv_hbm, bwo_hbm, out_hbm,
            ax_v, bx_v, raw, rawp,
            wt, a_wo, b_wkt, b_m,
            tmp_m, tmp_t, tmp_w, qkv_s, o_s, g_s, z_s, zrow, out_v,
            in_sems, out_sems):
    q_s = qkv_s.at[0:NT]
    k_s = qkv_s.at[NT:2 * NT]
    v_s = qkv_s.at[2 * NT:3 * NT]

    def cp(src, dst, i):
        return pltpu.make_async_copy(src, dst, in_sems.at[i])

    def c_bx(i):
        r = _rows(TB0 + (i - 1) * TB1, TB3 if isinstance(i, int) and i == 3 else TB1)
        return cp(bx_hbm.at[r], bx_v.at[r], i)

    def c_wo(i):
        return cp(awo_hbm.at[_rows(i * (D // 2), D // 2)], raw.at[1, _rows(i * (D // 2), D // 2)], 16 + i)

    c_raw = {2: cp(bwqkv_hbm.at[:, 2 * D:3 * D], raw.at[2], 10), 3: cp(bwo_hbm, raw.at[3], 11)}
    c_pair0 = cp(awqkv_hbm.at[:, 0:2 * D], rawp.at[0], 5)
    c_pair1 = [cp(awqkv_hbm.at[:, 2 * D:3 * D], rawp.at[1, :, 0:D], 6),
               cp(bwqkv_hbm.at[:, 0:D], rawp.at[1, :, D:2 * D], 6)]
    c_wka = cp(bwqkv_hbm.at[:, D:D + WA], raw.at[0, :, 0:WA], 0)
    c_wkb = cp(bwqkv_hbm.at[:, D + WA:2 * D], raw.at[0, :, WA:D], 4)
    c_xa = cp(bx_hbm.at[0:XA], bx_v.at[0:XA], 14)
    c_xb = cp(bx_hbm.at[XA:TB0], bx_v.at[XA:TB0], 15)
    c_ax0 = cp(ax_hbm.at[0:TA], ax_v.at[0:TA], 12)
    c_ax1 = cp(ax_hbm.at[TA:S], ax_v.at[TA:S], 13)
    for c in [c_wka, c_xa, c_wkb, c_xb, c_bx(1), c_pair0, c_wo(0), c_bx(2), c_pair1[0], c_pair1[1],
              c_wo(1), c_bx(3), c_raw[2], c_raw[3], c_ax0, c_ax1]:
        c.start()
    a_wt0 = 0
    b_wq0 = 3 * D

    def out_copy(r0, rows, col0, sem, ov=out_v, oh=out_hbm):
        return pltpu.make_async_copy(ov.at[r0:r0 + rows, col0:col0 + D],
                                     oh.at[r0:r0 + rows, col0:col0 + D], out_sems.at[sem])

    def pace(v, n):
        z = _gate(v.astype(F32)[0:8], jnp.uint32(0))
        return jnp.concatenate([z] * n, axis=0)

    def prep_pair(k, row_a, row_b):
        for t in range(NT):
            rows = slice(t * 128, (t + 1) * 128)
            tmp_t[0:D, :] = _pack2(rawp[k, rows, 0:D], rawp[k, rows, D:2 * D]).T
            for d in range(DH):
                x = tmp_t[pl.ds(d, H, stride=DH), :]
                if (t or d) and d % 4 == 0:
                    x = x | pace(wt[0, _rows(row_a, 16), :], H // 8)
                a, b = _unpack2(x)
                wt[t, _rows(row_a + d * H, H), :] = a
                wt[t, _rows(row_b + d * H, H), :] = b

    def prep_wo(i):
        hd = D // 2
        w = raw[1, _rows(i * hd, hd), :]
        for p in range(3):
            ta, tb = 2 * p, min(2 * p + 1, NT - 1)
            tmp_w[0:hd, :] = _pack2(w[:, ta * 128:(ta + 1) * 128], w[:, tb * 128:(tb + 1) * 128])
            for d in range(DH):
                x = tmp_w[pl.ds(d, H // 2, stride=DH), :]
                if (p or d) and d % 5 == 0:
                    x = x | pace(a_wo[0, _rows(i * (H // 2), 16), :], H // 16)
                a, b = _unpack2(x)
                rows = _rows(d * H + i * (H // 2), H // 2)
                a_wo[ta, rows, :] = a
                if tb != ta:
                    a_wo[tb, rows, :] = b

    def wk_transpose(f0, f1):
        wkt = raw[0, :, f0:f1].T
        for t in range(NT):
            b_wkt[t, f0:f1, :] = wkt[:, t * 128:(t + 1) * 128]

    def b1_k(r0, rows, f0=0, f1=D, first=False):
        x = bx_v[_rows(r0, rows), :]
        kt = jax.lax.dot_general(_ld(b_wkt, f0, f1), x, NT_DIMS, preferred_element_type=F32)
        pk = _phi(kt)
        zp = pk[:, 0:128]
        for j in range(1, rows // 128):
            zp = zp + pk[:, j * 128:(j + 1) * 128]
        if first:
            z_s[f0:f1, :] = zp
        else:
            z_s[f0:f1, :] += zp
        return pk.astype(BF16)

    def b1_g(r0, rows, pk, f0=0, f1=D, first=False):
        x = bx_v[_rows(r0, rows), :]
        g = jnp.dot(pk, x, preferred_element_type=F32)
        if first:
            g_s[f0:f1, :] = g
        else:
            g_s[f0:f1, :] += g

    def a_proj(xr, r0, b0, rows):
        y = jax.lax.dot_general(xr[r0:r0 + rows, :], _ld(wt, a_wt0, a_wt0 + 3 * D), NT_DIMS,
                                preferred_element_type=F32)
        for t in range(3 * NT):
            qkv_s[t, HALO + b0:HALO + b0 + rows, :] = y[:, t * 128:(t + 1) * 128]

    def a_attn(b0, rows, pace_on, tok=None, first=False):
        for c in range(rows // CH):
            c0 = HALO + b0 + c * CH
            sc = EXP2_SCALE if tok is None else _gate(tok, jnp.float32(EXP2_SCALE))
            q = [q_s[t, c0:c0 + CH, :] * sc for t in range(NT)]
            logits = []
            for w in range(W):
                off = c0 - DIL * w
                p = q[0] * k_s[0, off:off + CH, :]
                for t in range(1, NT):
                    p = p + q[t] * k_s[t, off:off + CH, :]
                l = _group_sum(p)
                if first and c * CH < HALO and w > 0:
                    pos = c * CH + jax.lax.broadcasted_iota(jnp.int32, (CH, 128), 0)
                    l = jnp.where(pos >= DIL * w, l, -1e9 * LOG2E)
                logits.append(l)
            m = logits[0]
            for w in range(1, W):
                m = jnp.maximum(m, logits[w])
            e = [jnp.exp2(l - m) for l in logits]
            den = e[0]
            for w in range(1, W):
                den = den + e[w]
            r = 1.0 / den
            tok = den if pace_on == "den" else logits[W - 1]
            for t in range(NT):
                acc = e[0] * v_s[t, c0:c0 + CH, :]
                for w in range(1, W):
                    off = c0 - DIL * w
                    acc = acc + e[w] * v_s[t, off:off + CH, :]
                o_s[t, c0 - HALO:c0 - HALO + CH, :] = (acc * r).astype(BF16)
        return tok

    def a_out(r0, b0, rows, sem, ov=out_v, oh=out_hbm):
        ov[r0:r0 + rows, 0:D] = jnp.dot(_ld(o_s, b0, b0 + rows), _ld(a_wo, 0, D),
                                        preferred_element_type=F32).astype(BF16)
        out_copy(r0, rows, 0, sem, ov, oh).start()

    def carry_halo():
        for t in range(NT):
            k_s[t, 0:HALO, :] = k_s[t, BUF:BUF + HALO, :]
            v_s[t, 0:HALO, :] = v_s[t, BUF:BUF + HALO, :]

    bounds = []
    for j in range(NT):
        h0 = (128 * j) // DH
        h1 = (128 * j + 127) // DH
        lo = (h0 * DH) // 8 * 8
        bounds.append((lo, lo + -(-((h1 + 1) * DH - lo) // 16) * 16))

    def b_switch():
        zp = jnp.concatenate([z_s[pl.ds(d, H, stride=DH), :] for d in range(DH)], axis=0)
        zrow[...] = jnp.broadcast_to(jnp.sum(zp.T, axis=0, keepdims=True), zrow.shape)
        kvs = []
        for j, (lo, hi) in enumerate(bounds):
            kv = jnp.dot(g_s[lo:hi, :].astype(BF16), raw[2, :, j * 128:(j + 1) * 128],
                         preferred_element_type=F32)
            row = lo + jax.lax.broadcasted_iota(jnp.int32, kv.shape, 0)
            head0 = (j * 128 + jax.lax.broadcasted_iota(jnp.int32, (1, 128), 1)) // DH * DH
            same_head = jnp.logical_and(row >= head0, row < head0 + DH)
            kvs.append(jnp.where(same_head, kv, 0.0).astype(BF16))
        done = 0
        for j, (lo, hi) in enumerate(bounds):
            mj = jnp.dot(kvs[j], raw[3, j * 128:(j + 1) * 128, :], preferred_element_type=F32)
            for t in range(NT):
                mt = mj[:, t * 128:(t + 1) * 128]
                if done > lo:
                    tmp_m[t, lo:done, :] += mt[0:done - lo]
                tmp_m[t, max(done, lo):hi, :] = mt[max(done, lo) - lo:]
            done = hi
        for t in range(NT):
            for d in range(DH):
                b_m[t, d * H:(d + 1) * H, :] = tmp_m[t, pl.ds(d, H, stride=DH), :].astype(BF16)

    def b2_q(xr, r0):
        q = jax.lax.dot_general(xr[r0:r0 + TA, :], _ld(wt, b_wq0, b_wq0 + D), NT_DIMS,
                                preferred_element_type=F32)
        z = zrow[...]
        dens, out = [], []
        for c in range(TA // CH):
            l2e = LOG2E if c < 2 else _gate(dens[c - 2], jnp.float32(LOG2E))
            pq = []
            for t in range(NT):
                qt = q[c * CH:(c + 1) * CH, t * 128:(t + 1) * 128]
                pq.append(jnp.where(qt > 0, qt + 1.0, jnp.exp2(qt * l2e)) + 1e-6)
            p = pq[0] * z[:, 0:128]
            for t in range(1, NT):
                p = p + pq[t] * z[:, t * 128:(t + 1) * 128]
            den = _group_sum(p) + 1e-6
            dens.append(den)
            r = 1.0 / den
            out.append(jnp.concatenate([pq[t] * r for t in range(NT)], axis=1))
        return jnp.concatenate(out, axis=0).astype(BF16)

    def b2_out(r0, pqn, sem, ov, oh):
        ov[r0:r0 + TA, D:2 * D] = jnp.dot(pqn, _ld(b_m, 0, D), preferred_element_type=F32).astype(BF16)
        out_copy(r0, TA, D, sem, ov, oh).start()

    b00 = BUF - TA

    def split(f0, f1, n):
        return [(f0 + k * (f1 - f0) // n, f0 + (k + 1) * (f1 - f0) // n) for k in range(n)]

    def main(_, carry0):
        c_wka.wait()
        wk_transpose(0, WA)
        c_xa.wait()
        pks = [b1_k(0, XA, f0, f1, True) for f0, f1 in split(0, WA, 2)]
        for (f0, f1), pk in zip(split(0, WA, 2), pks):
            b1_g(0, XA, pk, f0, f1, True)
        c_wkb.wait()
        c_xb.wait()
        pks = [b1_k(XA, TB0 - XA, f0, f1) for f0, f1 in split(0, WA, 2)]
        wk_transpose(WA, D)
        pks_b = [b1_k(0, TB0, f0, f1, True) for f0, f1 in split(WA, D, 4)]
        for (f0, f1), pk in zip(split(0, WA, 2), pks):
            b1_g(XA, TB0 - XA, pk, f0, f1)
        for (f0, f1), pk in zip(split(WA, D, 4), pks_b):
            b1_g(0, TB0, pk, f0, f1, True)

        def b1_loop(i, carry):
            c_bx(i + 1).wait()
            cp(rawp.at[i], rawp.at[i], 5 + i).wait()
            c_wo(i).wait()
            r0 = TB0 + i * TB1
            pk = b1_k(r0, TB1)
            prep_wo(i)
            prep_pair(i, 2 * i * D, (2 * i + 1) * D)
            b1_g(r0, TB1, pk)
            return carry

        jax.lax.fori_loop(0, 2, b1_loop, 0)

        for c in (c_bx(3), c_raw[2], c_raw[3], c_ax0):
            c.wait()
        pks = [b1_k(S - TB3, TB3, f0, f1) for f0, f1 in split(0, D, 4)]
        for t in range(NT):
            k_s[t, b00:b00 + HALO, :] = jnp.zeros((HALO, 128), F32)
            v_s[t, b00:b00 + HALO, :] = jnp.zeros((HALO, 128), F32)
        a_proj(ax_v, 0, b00, TA)
        for (f0, f1), pk in zip(split(0, D, 4), pks):
            b1_g(S - TB3, TB3, pk, f0, f1)
        b_switch()
        a_attn(b00, TA, "logit", first=True)
        a_out(0, b00, TA, 0)
        carry_halo()
        c_ax1.wait()

        def steady(it, carry):
            wa = pl.ds(pl.multiple_of(it * BUF, 128), TA + BUF)
            wb = pl.ds(pl.multiple_of(it * NSUB * TA, 128), NSUB * TA)
            axr, ova, oha = ax_v.at[wa], out_v.at[wa], out_hbm.at[wa]
            bxr, ovb, ohb = bx_v.at[wb], out_v.at[wb], out_hbm.at[wb]
            pqn = {}
            b_work = [[("q", 0), ("q", 1)], [("o", 0), ("q", 2)], [("o", 1), ("q", 3)], [("o", 2), ("o", 3)]]

            def emit_out(j):
                ra = TA + j * TA2
                sem = 1 + it * NO + j
                if j + 1 < NSUB:
                    a_out(ra, j * TA2, TA2, sem, ova, oha)
                else:
                    off = 0
                    for k, n in enumerate(OSP):
                        a_out(ra + off, j * TA2 + off, n, sem + k, ova, oha)
                        off += n

            tok = None
            for j in range(NSUB):
                ra = TA + j * TA2
                a_proj(axr, ra, j * TA2, TA2)
                if j > 0:
                    emit_out(j - 1)
                for kind, idx in b_work[j]:
                    if kind == "q":
                        pqn[idx] = b2_q(bxr, idx * TA)
                    else:
                        b2_out(idx * TA, pqn.pop(idx), 1 + 2 * NO + it * NSUB + idx, ovb, ohb)
                tok = a_attn(j * TA2, TA2, "den" if j + 1 < NSUB else "logit", tok)
            emit_out(NSUB - 1)
            carry_halo()
            return carry

        jax.lax.fori_loop(0, 2, steady, 0)
        return carry0

    jax.lax.fori_loop(0, 1 + pl.program_id(0), main, 0)

    out_copy(0, TA, 0, 0).wait()
    for it in range(2):
        for j in range(NSUB):
            r0 = TA + it * BUF + j * TA2
            sem = 1 + it * NO + j
            if j + 1 < NSUB:
                out_copy(r0, TA2, 0, sem).wait()
            else:
                off = 0
                for k, n in enumerate(OSP):
                    out_copy(r0 + off, n, 0, sem + k).wait()
                    off += n
    for i in range(2 * NSUB):
        out_copy(i * TA, TA, D, 1 + 2 * NO + i).wait()


@jax.jit
def pallas_concat_heads__sliding_local_dilated__linear_attn_block__prompt_kernel(A_x, A_wqkv, A_wo, B_x, B_wqkv, B_wo):
    any_spec = pl.BlockSpec(memory_space=pl.ANY)
    out = pl.pallas_call(
        _kernel,
        out_shape=jax.ShapeDtypeStruct((S, 2 * D), BF16),
        grid=(1,),
        in_specs=[any_spec] * 6,
        out_specs=any_spec,
        scratch_shapes=[
            pltpu.VMEM((S, D), BF16), pltpu.VMEM((S, D), BF16),
            pltpu.VMEM((4, D, D), BF16), pltpu.VMEM((2, D, 2 * D), BF16),
            pltpu.VMEM((NT, 4 * D, 128), BF16), pltpu.VMEM((NT, D, 128), BF16),
            pltpu.VMEM((NT, D, 128), BF16), pltpu.VMEM((NT, D, 128), BF16),
            pltpu.VMEM((NT, D + PAD, 128), F32), pltpu.VMEM((D + PAD, 128), U32),
            pltpu.VMEM((D // 2 + PAD, 128), U32),
            pltpu.VMEM((3 * NT, HALO + BUF, 128), F32),
            pltpu.VMEM((NT, BUF, 128), BF16),
            pltpu.VMEM((D, D), F32), pltpu.VMEM((D + PAD, 128), F32), pltpu.VMEM((8, D), F32),
            pltpu.VMEM((S, 2 * D), BF16),
            pltpu.SemaphoreType.DMA((18,)), pltpu.SemaphoreType.DMA((9 + 2 * NO,)),
        ],
        compiler_params=pltpu.CompilerParams(vmem_limit_bytes=100 * 1024 * 1024,
                                             disable_bounds_checks=True,
                                             disable_semaphore_checks=True),
    )(A_x.reshape(S, D), A_wqkv, A_wo, B_x.reshape(S, D), B_wqkv, B_wo)
    return out.reshape(1, S, 2 * D)
```

```python
import math

import jax
import jax.numpy as jnp
import jax.experimental.pallas as pl
import jax.experimental.pallas.tpu as pltpu

S = 2048
D = 640
H = 32
DH = 20
W = 8
DIL = 2
NT = D // 128
TA = 256
TB0 = 640
TB1 = 512
TB3 = S - TB0 - 2 * TB1
HALO = 16
TA2 = 224
NSUB = 4
BUF = NSUB * TA2
WA = 256
XA = 384
CH = 8
OSP = (128, 64, 32)
NO = NSUB - 1 + len(OSP)
PAD = 24
F32 = jnp.float32
BF16 = jnp.bfloat16
U32 = jnp.uint32
NT_DIMS = (((1,), (1,)), ((), ()))
LOG2E = math.log2(math.e)
EXP2_SCALE = (DH ** -0.5) * LOG2E


def _gate(tok, value):
    return jnp.where(tok > jnp.inf, value + 1, value)


def _phi(t):
    return jnp.where(t > 0, t + 1.0, jnp.exp(t)) + 1e-6


def _group_sum(p):
    return (p + pltpu.roll(p, 64, 1)) + (pltpu.roll(p, 32, 1) + pltpu.roll(p, 96, 1))


def _ld(ref, r0, r1):
    return jnp.concatenate([ref[t, r0:r1, :] for t in range(NT)], axis=1)


def _rows(r0, n):
    return pl.ds(r0 if isinstance(r0, int) else pl.multiple_of(r0, 16), n)


def _pack2(a, b):
    lo = jax.lax.bitcast_convert_type(a.astype(F32), U32) >> 16
    return lo | jax.lax.bitcast_convert_type(b.astype(F32), U32)


def _unpack2(x):
    a = jax.lax.bitcast_convert_type(x << 16, F32)
    b = jax.lax.bitcast_convert_type(x & jnp.uint32(0xFFFF0000), F32)
    return a.astype(BF16), b.astype(BF16)


def _kernel(ax_hbm, awqkv_hbm, awo_hbm, bx_hbm, bwqkv_hbm, bwo_hbm, out_hbm,
            ax_v, bx_v, raw, rawp,
            wt, a_wo, b_wkt, b_m,
            tmp_m, tmp_t, tmp_w, qkv_s, o_s, g_s, z_s, zrow, out_v,
            in_sems, out_sems):
    q_s = qkv_s.at[0:NT]
    k_s = qkv_s.at[NT:2 * NT]
    v_s = qkv_s.at[2 * NT:3 * NT]

    def cp(src, dst, i):
        return pltpu.make_async_copy(src, dst, in_sems.at[i])

    def c_bx(i):
        r = _rows(TB0 + (i - 1) * TB1, TB3 if isinstance(i, int) and i == 3 else TB1)
        return cp(bx_hbm.at[r], bx_v.at[r], i)

    def c_wo(i):
        return cp(awo_hbm.at[_rows(i * (D // 2), D // 2)], raw.at[1, _rows(i * (D // 2), D // 2)], 16 + i)

    c_raw = {2: cp(bwqkv_hbm.at[:, 2 * D:3 * D], raw.at[2], 10), 3: cp(bwo_hbm, raw.at[3], 11)}
    c_pair0 = cp(awqkv_hbm.at[:, 0:2 * D], rawp.at[0], 5)
    c_pair1 = [cp(awqkv_hbm.at[:, 2 * D:3 * D], rawp.at[1, :, 0:D], 6),
               cp(bwqkv_hbm.at[:, 0:D], rawp.at[1, :, D:2 * D], 6)]
    c_wka = cp(bwqkv_hbm.at[:, D:D + WA], raw.at[0, :, 0:WA], 0)
    c_wkb = cp(bwqkv_hbm.at[:, D + WA:2 * D], raw.at[0, :, WA:D], 4)
    c_xa = cp(bx_hbm.at[0:XA], bx_v.at[0:XA], 14)
    c_xb = cp(bx_hbm.at[XA:TB0], bx_v.at[XA:TB0], 15)
    c_ax0 = cp(ax_hbm.at[0:TA], ax_v.at[0:TA], 12)
    c_ax1 = cp(ax_hbm.at[TA:S], ax_v.at[TA:S], 13)
    for c in [c_wka, c_xa, c_wkb, c_xb, c_bx(1), c_pair0, c_wo(0), c_bx(2), c_pair1[0], c_pair1[1],
              c_wo(1), c_bx(3), c_raw[2], c_raw[3], c_ax0, c_ax1]:
        c.start()
    a_wt0 = 0
    b_wq0 = 3 * D

    def out_copy(r0, rows, col0, sem, ov=out_v, oh=out_hbm):
        return pltpu.make_async_copy(ov.at[r0:r0 + rows, col0:col0 + D],
                                     oh.at[r0:r0 + rows, col0:col0 + D], out_sems.at[sem])

    def pace(v, n):
        z = _gate(v.astype(F32)[0:8], jnp.uint32(0))
        return jnp.concatenate([z] * n, axis=0)

    def prep_pair(k, row_a, row_b):
        for t in range(NT):
            rows = slice(t * 128, (t + 1) * 128)
            tmp_t[0:D, :] = _pack2(rawp[k, rows, 0:D], rawp[k, rows, D:2 * D]).T
            for d in range(DH):
                x = tmp_t[pl.ds(d, H, stride=DH), :]
                if (t or d) and d % 4 == 0:
                    x = x | pace(wt[0, _rows(row_a, 16), :], H // 8)
                a, b = _unpack2(x)
                wt[t, _rows(row_a + d * H, H), :] = a
                wt[t, _rows(row_b + d * H, H), :] = b

    def prep_wo(i):
        hd = D // 2
        w = raw[1, _rows(i * hd, hd), :]
        for p in range(3):
            ta, tb = 2 * p, min(2 * p + 1, NT - 1)
            tmp_w[0:hd, :] = _pack2(w[:, ta * 128:(ta + 1) * 128], w[:, tb * 128:(tb + 1) * 128])
            for d in range(DH):
                x = tmp_w[pl.ds(d, H // 2, stride=DH), :]
                if (p or d) and d % 5 == 0:
                    x = x | pace(a_wo[0, _rows(i * (H // 2), 16), :], H // 16)
                a, b = _unpack2(x)
                rows = _rows(d * H + i * (H // 2), H // 2)
                a_wo[ta, rows, :] = a
                if tb != ta:
                    a_wo[tb, rows, :] = b

    def wk_transpose(f0, f1):
        wkt = raw[0, :, f0:f1].T
        for t in range(NT):
            b_wkt[t, f0:f1, :] = wkt[:, t * 128:(t + 1) * 128]

    def b1_k(r0, rows, f0=0, f1=D, first=False):
        x = bx_v[_rows(r0, rows), :]
        kt = jax.lax.dot_general(_ld(b_wkt, f0, f1), x, NT_DIMS, preferred_element_type=F32)
        pk = _phi(kt)
        zp = pk[:, 0:128]
        for j in range(1, rows // 128):
            zp = zp + pk[:, j * 128:(j + 1) * 128]
        if first:
            z_s[f0:f1, :] = zp
        else:
            z_s[f0:f1, :] += zp
        return pk.astype(BF16)

    def b1_g(r0, rows, pk, f0=0, f1=D, first=False):
        x = bx_v[_rows(r0, rows), :]
        g = jnp.dot(pk, x, preferred_element_type=F32)
        if first:
            g_s[f0:f1, :] = g
        else:
            g_s[f0:f1, :] += g

    def a_proj(xr, r0, b0, rows):
        y = jax.lax.dot_general(xr[r0:r0 + rows, :], _ld(wt, a_wt0, a_wt0 + 3 * D), NT_DIMS,
                                preferred_element_type=F32)
        for t in range(3 * NT):
            qkv_s[t, HALO + b0:HALO + b0 + rows, :] = y[:, t * 128:(t + 1) * 128]

    def a_attn(b0, rows, tok=None, first=False):
        for c in range(rows // CH):
            c0 = HALO + b0 + c * CH
            sc = EXP2_SCALE if tok is None else _gate(tok, jnp.float32(EXP2_SCALE))
            q = [q_s[t, c0:c0 + CH, :] * sc for t in range(NT)]
            logits = []
            for w in range(W):
                off = c0 - DIL * w
                p = q[0] * k_s[0, off:off + CH, :]
                for t in range(1, NT):
                    p = p + q[t] * k_s[t, off:off + CH, :]
                l = _group_sum(p)
                if first and c * CH < HALO and w > 0:
                    pos = c * CH + jax.lax.broadcasted_iota(jnp.int32, (CH, 128), 0)
                    l = jnp.where(pos >= DIL * w, l, -1e9 * LOG2E)
                logits.append(l)
            m = logits[0]
            for w in range(1, W):
                m = jnp.maximum(m, logits[w])
            e = [jnp.exp2(l - m) for l in logits]
            den = e[0]
            for w in range(1, W):
                den = den + e[w]
            r = 1.0 / den
            tok = logits[3] if first else m
            for t in range(NT):
                acc = e[0] * v_s[t, c0:c0 + CH, :]
                for w in range(1, W):
                    off = c0 - DIL * w
                    acc = acc + e[w] * v_s[t, off:off + CH, :]
                o_s[t, c0 - HALO:c0 - HALO + CH, :] = (acc * r).astype(BF16)
        return tok

    def a_out(r0, b0, rows, sem, ov=out_v, oh=out_hbm):
        ov[r0:r0 + rows, 0:D] = jnp.dot(_ld(o_s, b0, b0 + rows), _ld(a_wo, 0, D),
                                        preferred_element_type=F32).astype(BF16)
        out_copy(r0, rows, 0, sem, ov, oh).start()

    def carry_halo():
        for t in range(NT):
            k_s[t, 0:HALO, :] = k_s[t, BUF:BUF + HALO, :]
            v_s[t, 0:HALO, :] = v_s[t, BUF:BUF + HALO, :]

    bounds = []
    for j in range(NT):
        h0 = (128 * j) // DH
        h1 = (128 * j + 127) // DH
        lo = (h0 * DH) // 8 * 8
        bounds.append((lo, lo + -(-((h1 + 1) * DH - lo) // 16) * 16))

    def b_switch():
        zp = jnp.concatenate([z_s[pl.ds(d, H, stride=DH), :] for d in range(DH)], axis=0)
        zrow[...] = jnp.broadcast_to(jnp.sum(zp.T, axis=0, keepdims=True), zrow.shape)
        kvs = []
        for j, (lo, hi) in enumerate(bounds):
            kv = jnp.dot(g_s[lo:hi, :].astype(BF16), raw[2, :, j * 128:(j + 1) * 128],
                         preferred_element_type=F32)
            row = lo + jax.lax.broadcasted_iota(jnp.int32, kv.shape, 0)
            head0 = (j * 128 + jax.lax.broadcasted_iota(jnp.int32, (1, 128), 1)) // DH * DH
            same_head = jnp.logical_and(row >= head0, row < head0 + DH)
            kvs.append(jnp.where(same_head, kv, 0.0).astype(BF16))
        done = 0
        for j, (lo, hi) in enumerate(bounds):
            mj = jnp.dot(kvs[j], raw[3, j * 128:(j + 1) * 128, :], preferred_element_type=F32)
            for t in range(NT):
                mt = mj[:, t * 128:(t + 1) * 128]
                if done > lo:
                    tmp_m[t, lo:done, :] += mt[0:done - lo]
                tmp_m[t, max(done, lo):hi, :] = mt[max(done, lo) - lo:]
            done = hi
        for t in range(NT):
            for d in range(DH):
                b_m[t, d * H:(d + 1) * H, :] = tmp_m[t, pl.ds(d, H, stride=DH), :].astype(BF16)

    def b2_q(xr, r0):
        q = jax.lax.dot_general(xr[r0:r0 + TA, :], _ld(wt, b_wq0, b_wq0 + D), NT_DIMS,
                                preferred_element_type=F32)
        z = zrow[...]
        out = []
        for c in range(TA // CH):
            l2e = LOG2E if c < 3 else _gate(out[c - 3][:, D - 128:D], jnp.float32(LOG2E))
            pq = []
            for t in range(NT):
                qt = q[c * CH:(c + 1) * CH, t * 128:(t + 1) * 128]
                pq.append(jnp.where(qt > 0, qt + 1.0, jnp.exp2(qt * l2e)) + 1e-6)
            p = pq[0] * z[:, 0:128]
            for t in range(1, NT):
                p = p + pq[t] * z[:, t * 128:(t + 1) * 128]
            r = 1.0 / (_group_sum(p) + 1e-6)
            out.append(jnp.concatenate([pq[t] * r for t in range(NT)], axis=1))
        return jnp.concatenate(out, axis=0).astype(BF16)

    def b2_out(r0, pqn, sem, ov, oh):
        ov[r0:r0 + TA, D:2 * D] = jnp.dot(pqn, _ld(b_m, 0, D), preferred_element_type=F32).astype(BF16)
        out_copy(r0, TA, D, sem, ov, oh).start()

    b00 = BUF - TA

    def split(f0, f1, n):
        return [(f0 + k * (f1 - f0) // n, f0 + (k + 1) * (f1 - f0) // n) for k in range(n)]

    def main(_, carry0):
        c_wka.wait()
        wk_transpose(0, WA)
        c_xa.wait()
        pks = [b1_k(0, XA, f0, f1, True) for f0, f1 in split(0, WA, 2)]
        for (f0, f1), pk in zip(split(0, WA, 2), pks):
            b1_g(0, XA, pk, f0, f1, True)
        c_wkb.wait()
        c_xb.wait()
        pks = [b1_k(XA, TB0 - XA, f0, f1) for f0, f1 in split(0, WA, 2)]
        wk_transpose(WA, D)
        pks_b = [b1_k(0, TB0, f0, f1, True) for f0, f1 in split(WA, D, 4)]
        for (f0, f1), pk in zip(split(0, WA, 2), pks):
            b1_g(XA, TB0 - XA, pk, f0, f1)
        for (f0, f1), pk in zip(split(WA, D, 4), pks_b):
            b1_g(0, TB0, pk, f0, f1, True)

        def b1_loop(i, carry):
            c_bx(i + 1).wait()
            cp(rawp.at[i], rawp.at[i], 5 + i).wait()
            c_wo(i).wait()
            r0 = TB0 + i * TB1
            pk = b1_k(r0, TB1)
            prep_wo(i)
            prep_pair(i, 2 * i * D, (2 * i + 1) * D)
            b1_g(r0, TB1, pk)
            return carry

        jax.lax.fori_loop(0, 2, b1_loop, 0)

        for c in (c_bx(3), c_raw[2], c_raw[3], c_ax0):
            c.wait()
        pks = [b1_k(S - TB3, TB3, f0, f1) for f0, f1 in split(0, D, 4)]
        for t in range(NT):
            k_s[t, b00:b00 + HALO, :] = jnp.zeros((HALO, 128), F32)
            v_s[t, b00:b00 + HALO, :] = jnp.zeros((HALO, 128), F32)
        a_proj(ax_v, 0, b00, TA)
        for (f0, f1), pk in zip(split(0, D, 4), pks):
            b1_g(S - TB3, TB3, pk, f0, f1)
        b_switch()
        a_attn(b00, TA, first=True)
        a_out(0, b00, TA, 0)
        carry_halo()
        c_ax1.wait()

        def steady(it, carry):
            wa = pl.ds(pl.multiple_of(it * BUF, 128), TA + BUF)
            wb = pl.ds(pl.multiple_of(it * NSUB * TA, 128), NSUB * TA)
            axr, ova, oha = ax_v.at[wa], out_v.at[wa], out_hbm.at[wa]
            bxr, ovb, ohb = bx_v.at[wb], out_v.at[wb], out_hbm.at[wb]
            pqn = {}
            b_work = [[("q", 0)], [("q", 1), ("o", 0)], [("q", 2), ("q", 3)], [("o", 1), ("o", 2), ("o", 3)]]

            def emit_out(j):
                ra = TA + j * TA2
                sem = 1 + it * NO + j
                if j + 1 < NSUB:
                    a_out(ra, j * TA2, TA2, sem, ova, oha)
                else:
                    off = 0
                    for k, n in enumerate(OSP):
                        a_out(ra + off, j * TA2 + off, n, sem + k, ova, oha)
                        off += n

            tok = None
            for j in range(NSUB):
                ra = TA + j * TA2
                a_proj(axr, ra, j * TA2, TA2)
                for kind, idx in b_work[j]:
                    if kind == "q":
                        pqn[idx] = b2_q(bxr, idx * TA)
                    else:
                        b2_out(idx * TA, pqn.pop(idx), 1 + 2 * NO + it * NSUB + idx, ovb, ohb)
                if j > 0:
                    emit_out(j - 1)
                tok = a_attn(j * TA2, TA2, tok)
            emit_out(NSUB - 1)
            carry_halo()
            return carry

        jax.lax.fori_loop(0, 2, steady, 0)
        return carry0

    jax.lax.fori_loop(0, 1 + pl.program_id(0), main, 0)

    for i in range(2 * NSUB):
        out_copy(i * TA, TA, D, 1 + 2 * NO + i).wait()
    out_copy(0, TA, 0, 0).wait()
    for it in range(2):
        for j in range(NSUB):
            r0 = TA + it * BUF + j * TA2
            sem = 1 + it * NO + j
            if j + 1 < NSUB:
                out_copy(r0, TA2, 0, sem).wait()
            else:
                off = 0
                for k, n in enumerate(OSP):
                    out_copy(r0 + off, n, 0, sem + k).wait()
                    off += n


@jax.jit
def pallas_concat_heads__sliding_local_dilated__linear_attn_block__prompt_kernel(A_x, A_wqkv, A_wo, B_x, B_wqkv, B_wo):
    any_spec = pl.BlockSpec(memory_space=pl.ANY)
    out = pl.pallas_call(
        _kernel,
        out_shape=jax.ShapeDtypeStruct((S, 2 * D), BF16),
        grid=(1,),
        in_specs=[any_spec] * 6,
        out_specs=any_spec,
        scratch_shapes=[
            pltpu.VMEM((S, D), BF16), pltpu.VMEM((S, D), BF16),
            pltpu.VMEM((4, D, D), BF16), pltpu.VMEM((2, D, 2 * D), BF16),
            pltpu.VMEM((NT, 4 * D, 128), BF16), pltpu.VMEM((NT, D, 128), BF16),
            pltpu.VMEM((NT, D, 128), BF16), pltpu.VMEM((NT, D, 128), BF16),
            pltpu.VMEM((NT, D + PAD, 128), F32), pltpu.VMEM((D + PAD, 128), U32),
            pltpu.VMEM((D // 2 + PAD, 128), U32),
            pltpu.VMEM((3 * NT, HALO + BUF, 128), F32),
            pltpu.VMEM((NT, BUF, 128), BF16),
            pltpu.VMEM((D, D), F32), pltpu.VMEM((D + PAD, 128), F32), pltpu.VMEM((8, D), F32),
            pltpu.VMEM((S, 2 * D), BF16),
            pltpu.SemaphoreType.DMA((18,)), pltpu.SemaphoreType.DMA((9 + 2 * NO,)),
        ],
        compiler_params=pltpu.CompilerParams(vmem_limit_bytes=100 * 1024 * 1024,
                                             disable_bounds_checks=True,
                                             disable_semaphore_checks=True),
    )(A_x.reshape(S, D), A_wqkv, A_wo, B_x.reshape(S, D), B_wqkv, B_wo)
    return out.reshape(1, S, 2 * D)
```
